```python
import os as _os
_os.environ.setdefault("JAX_PLATFORMS", "cpu")
import jax
import jax.numpy as jnp

def _softmax(x, axis=-1):
    return jax.nn.softmax(x, axis=axis)
def _gelu(x):
    return jax.nn.gelu(x, approximate=True)
def _silu(x):
    return jax.nn.silu(x)
def _sigmoid(x):
    return jax.nn.sigmoid(x)
def _layernorm(x, axis=-1, eps=1e-5):
    m = jnp.mean(x, axis=axis, keepdims=True)
    v = jnp.var(x, axis=axis, keepdims=True)
    return (x - m) / jnp.sqrt(v + eps)
def _scatter_add(tgt, idx, src, axis=0):
    return tgt.at[idx].add(src)
def _segment_sum(src, seg, n):
    return jax.ops.segment_sum(src, seg, n)
class _Rng:
    def __init__(self, key):
        self._k = key
    def _next(self):
        self._k, sub = jax.random.split(self._k)
        return sub
    def normal(self, shape):
        return jax.random.normal(self._next(), shape, dtype=jnp.bfloat16)
    def randint(self, lo, hi, shape):
        return jax.random.randint(self._next(), shape, lo, hi, dtype=jnp.int32)
    def uniform(self, shape, lo=0.0, hi=1.0):
        return jax.random.uniform(self._next(), shape, jnp.bfloat16, lo, hi)
    def permutation(self, n):
        return jax.random.permutation(self._next(), n)


kernel_name = 'concat_heads__sliding_block_cached__sliding_block_cached__decode'

def setup_inputs():
    _rng = _Rng(jax.random.key(int.from_bytes(__import__("os").urandom(4), "little")))
    _w = (lambda a: (lambda t: t.astype(jnp.bfloat16) if jnp.issubdtype(t.dtype, jnp.floating) else t)(jnp.asarray(a)))
    def _A_setup():
        B, Sq, D = 4, 1, 576
        Hq, Hkv, Sk, Dh = 32, 16, 8192, 128
        assert Hq % Hkv == 0, (Hq, Hkv)
        return {
            "x": _w((lambda *s: _rng.normal(s) * 0.8)(B, Sq, D)),
            "k_cache": _w((lambda *s: _rng.normal(s) * 0.8)(B, Hkv, Sk, Dh)),
            "v_cache": _w((lambda *s: _rng.normal(s) * 0.05)(B, Hkv, Sk, Dh)),
            "wq": _w((lambda *s: _rng.normal(s) * 0.8)(D, Hq * Dh) * (D ** -0.5)),
            "wo": _w((lambda *s: _rng.normal(s) * 0.05)(Hq * Dh, D) * ((Hq * Dh) ** -0.5)),
        }
    _A_in = _A_setup()

    def _B_setup():
        B, Sq, D = 4, 1, 576
        Hq, Hkv, Sk, Dh = 32, 16, 8192, 128
        assert Hq % Hkv == 0, (Hq, Hkv)
        return {
            "x": _w((lambda *s: _rng.normal(s) * 0.8)(B, Sq, D)),
            "k_cache": _w((lambda *s: _rng.normal(s) * 0.8)(B, Hkv, Sk, Dh)),
            "v_cache": _w((lambda *s: _rng.normal(s) * 0.05)(B, Hkv, Sk, Dh)),
            "wq": _w((lambda *s: _rng.normal(s) * 0.8)(D, Hq * Dh) * (D ** -0.5)),
            "wo": _w((lambda *s: _rng.normal(s) * 0.05)(Hq * Dh, D) * ((Hq * Dh) ** -0.5)),
        }
    _B_in = _B_setup()

    return {
        "A_x": _A_in["x"],
        "A_k_cache": _A_in["k_cache"],
        "A_v_cache": _A_in["v_cache"],
        "A_wq": _A_in["wq"],
        "A_wo": _A_in["wo"],
        "B_x": _B_in["x"],
        "B_k_cache": _B_in["k_cache"],
        "B_v_cache": _B_in["v_cache"],
        "B_wq": _B_in["wq"],
        "B_wo": _B_in["wo"],
    }

def reference(A_x, A_k_cache, A_v_cache, A_wq, A_wo, B_x, B_k_cache, B_v_cache, B_wq, B_wo):
    def _A_ref(x, k_cache, v_cache, wq, wo):
        B, Sq, D = x.shape
        Hq, Dh = 32, 128
        Hkv, Sk = k_cache.shape[1], k_cache.shape[2]
        W = min(4096, max(256, Sk // 4))
        rep = Hq // Hkv
        q = (lambda x, *d: x.transpose(*d))((x @ wq).reshape(B, Sq, Hq, Dh), 0, 2, 1, 3)
        k = jnp.repeat(k_cache[:, :, Sk - W:, :], rep, axis=1)
        v = jnp.repeat(v_cache[:, :, Sk - W:, :], rep, axis=1)
        scores = jnp.einsum("bhqd,bhkd->bhqk", q, k) * (Dh ** -0.5)
        p = _softmax(scores, axis=-1)
        o = jnp.einsum("bhqk,bhkd->bhqd", p, v)
        return (lambda x, *d: x.transpose(*d))(o, 0, 2, 1, 3).reshape(B, Sq, Hq * Dh) @ wo

    def _B_ref(x, k_cache, v_cache, wq, wo):
        B, Sq, D = x.shape
        Hq, Dh = 32, 128
        Hkv, Sk = k_cache.shape[1], k_cache.shape[2]
        W = min(4096, max(256, Sk // 4))
        rep = Hq // Hkv
        q = (lambda x, *d: x.transpose(*d))((x @ wq).reshape(B, Sq, Hq, Dh), 0, 2, 1, 3)
        k = jnp.repeat(k_cache[:, :, Sk - W:, :], rep, axis=1)
        v = jnp.repeat(v_cache[:, :, Sk - W:, :], rep, axis=1)
        scores = jnp.einsum("bhqd,bhkd->bhqk", q, k) * (Dh ** -0.5)
        p = _softmax(scores, axis=-1)
        o = jnp.einsum("bhqk,bhkd->bhqd", p, v)
        return (lambda x, *d: x.transpose(*d))(o, 0, 2, 1, 3).reshape(B, Sq, Hq * Dh) @ wo

    a = _A_ref(A_x, A_k_cache, A_v_cache, A_wq, A_wo)
    b = _B_ref(B_x, B_k_cache, B_v_cache, B_wq, B_wo)
    return jnp.concatenate([a, b], axis=-1)
```

```python
import functools
import jax
import jax.numpy as jnp
from jax import lax
from jax.experimental import pallas as pl
from jax.experimental.pallas import tpu as pltpu

_NT = (((1,), (1,)), ((), ()))
_NN = (((1,), (0,)), ((), ()))


def make(LAG=3, NBUF=4, CH=128, split_issue=True, last_split=4):
    HQ, DH = 32, 128

    def fn(A_x, A_k, A_v, A_wq, A_wo, B_x, B_k, B_v, B_wq, B_wo):
        B, Sq, D = A_x.shape
        Hkv, Sk = A_k.shape[1], A_k.shape[2]
        W = min(4096, max(256, Sk // 4))
        S0 = Sk - W
        F = HQ * DH
        WC = 1024
        WR = 16
        NCB = F // WC
        NI = B * Hkv
        NOUT = 2 * D // 128
        scale = DH ** -0.5

        def kern(ax, ak, av, awq, awo, bx, bk, bv, bwq, bwo, o_ref,
                 xbuf, wqbuf, wobuf, kbuf, vbuf, qs, os_, xsem, wqsem, wosem, kvsem):
            def wq_start(u):
                br, c = divmod(u, NCB)
                src = (awq, bwq)[br]
                def body(r, _):
                    for p in range(2):
                        r0 = pl.multiple_of((2 * r + p) * WR, WR)
                        pltpu.make_async_copy(
                            src.at[pl.ds(r0, WR), pl.ds(c * WC, WC)],
                            wqbuf.at[br, pl.ds(r0, WR), pl.ds(c * WC, WC)],
                            wqsem.at[u]).start(priority=p)
                    return _
                lax.fori_loop(0, D // WR // 2, body, 0)

            def wq_wait(u):
                br, c = divmod(u, NCB)
                dst = wqbuf.at[br, :, pl.ds(c * WC, WC)]
                pltpu.make_async_copy(dst, dst, wqsem.at[u]).wait()

            def kv_start(kk, vv, i, lo, hi):
                b = i % B
                h = i // B
                slot = i % NBUF
                for c in range(lo, hi):
                    pltpu.make_async_copy(kk.at[b, h, pl.ds(S0 + c * CH, CH), :],
                                          kbuf.at[slot, pl.ds(c * CH, CH), :],
                                          kvsem.at[0, slot]).start(priority=0)
                    pltpu.make_async_copy(vv.at[b, h, pl.ds(S0 + c * CH, CH), :],
                                          vbuf.at[slot, pl.ds(c * CH, CH), :],
                                          kvsem.at[1, slot]).start(priority=1)

            def wo_start(u):
                n = 0
                for c in range(NCB):
                    for r in range(u * 128, (u + 1) * 128, WR):
                        br, rr = divmod(r, D)
                        pltpu.make_async_copy(
                            (awo, bwo)[br].at[pl.ds(rr, WR), pl.ds(c * WC, WC)],
                            wobuf.at[pl.ds(r, WR), pl.ds(c * WC, WC)],
                            wosem.at[u, c]).start(priority=n % 2)
                        n += 1

            def wo_wait(u, c):
                dst = wobuf.at[pl.ds(u * 128, 128), pl.ds(c * WC, WC)]
                pltpu.make_async_copy(dst, dst, wosem.at[u, c]).wait()

            NC = W // CH
            def q_compute(u):
                br, c = divmod(u, NCB)
                wq_wait(u)
                q = lax.dot_general(xbuf[br], wqbuf[br, :, pl.ds(c * WC, WC)], _NN,
                                    preferred_element_type=jnp.float32)
                for t in range(WC // DH):
                    qs[c * (WC // DH) + t, pl.ds(br * B, B), :] = q[:, t * DH:(t + 1) * DH]

            def attend(g, mid):
                slot = g % NBUF
                row = (g // NI) * B + g % B
                h = (g % NI) // B
                sub = lax.broadcasted_iota(jnp.int32, (8, DH), 0)
                q0 = jnp.broadcast_to(qs[2 * h, pl.ds(row, 1), :], (8, DH))
                q1 = jnp.broadcast_to(qs[2 * h + 1, pl.ds(row, 1), :], (8, DH))
                q = jnp.where(sub < 4, q0, q1).astype(jnp.bfloat16)
                pltpu.make_async_copy(kbuf.at[slot], kbuf.at[slot], kvsem.at[0, slot]).wait()
                s = lax.dot_general(q, kbuf[slot], _NT, preferred_element_type=jnp.float32) * scale
                m = jnp.max(s, axis=-1, keepdims=True)
                p = jnp.exp(s - m)
                l = jnp.sum(p, axis=-1, keepdims=True)
                mid()
                pltpu.make_async_copy(vbuf.at[slot], vbuf.at[slot], kvsem.at[1, slot]).wait()
                o = lax.dot_general(p.astype(jnp.bfloat16), vbuf[slot], _NN,
                                    preferred_element_type=jnp.float32) / l
                os_[2 * h, pl.ds(row, 1), :] = o[0:1]
                os_[2 * h + 1, pl.ds(row, 1), :] = o[4:5]

            def proj(u):
                acc = None
                for c in range(NCB):
                    wo_wait(u, c)
                    lhs = jnp.concatenate([os_[c * (WC // DH) + t] for t in range(WC // DH)], axis=1)
                    r = lax.dot_general(lhs.astype(jnp.bfloat16),
                                        wobuf[pl.ds(u * 128, 128), pl.ds(c * WC, WC)], _NT,
                                        preferred_element_type=jnp.float32)
                    acc = r if acc is None else acc + r
                lo, hi = acc[0:B], acc[B:2 * B]
                if (u + 1) * 128 <= D:
                    res = lo
                elif u * 128 >= D:
                    res = hi
                else:
                    lane = lax.broadcasted_iota(jnp.int32, (B, 128), 1)
                    res = jnp.where(lane < D - u * 128, lo, hi)
                o_ref[:, pl.ds(u * 128, 128)] = res.astype(o_ref.dtype)

            xc = [pltpu.make_async_copy(x, xbuf.at[i], xsem.at[i]) for i, x in enumerate((ax, bx))]
            NQ = 2 * NCB
            for u in range(NQ + LAG):
                if u < NQ:
                    wq_start(u)
                else:
                    kv_start(ak, av, u - NQ, 0, NC)
                if u == 0:
                    for c in xc:
                        c.start()
                if u == LAG:
                    for c in xc:
                        c.wait()
                if u >= LAG:
                    q_compute(u - LAG)

            def loop(kk, vv, lo, hi, off):
                def body(g, _):
                    if split_issue:
                        kv_start(kk, vv, g + off, 0, NC // 2)
                        attend(g, lambda: kv_start(kk, vv, g + off, NC // 2, NC))
                    else:
                        kv_start(kk, vv, g + off, 0, NC)
                        attend(g, lambda: None)
                    return _
                lax.fori_loop(lo, hi, body, 0)
            loop(ak, av, 0, NI - LAG, LAG)
            loop(bk, bv, NI - LAG, 2 * NI - LAG, LAG - NI)

            for u in range(NOUT + LAG):
                if u < NOUT:
                    wo_start(u)
                if u < LAG:
                    attend(2 * NI - LAG + u, lambda: None)
                else:
                    proj(u - LAG)

        hbm = pl.BlockSpec(memory_space=pltpu.HBM)
        out = pl.pallas_call(
            kern,
            out_shape=jax.ShapeDtypeStruct((B, 2 * D), A_x.dtype),
            in_specs=[hbm] * 10,
            out_specs=pl.BlockSpec(memory_space=pltpu.VMEM),
            scratch_shapes=[
                pltpu.VMEM((2, B, D), A_x.dtype),
                pltpu.VMEM((2, D, F), A_wq.dtype),
                pltpu.VMEM((2 * D, F), A_wo.dtype),
                pltpu.VMEM((NBUF, W, DH), A_k.dtype),
                pltpu.VMEM((NBUF, W, DH), A_v.dtype),
                pltpu.VMEM((HQ, 2 * B, DH), jnp.float32),
                pltpu.VMEM((HQ, 2 * B, DH), jnp.float32),
                pltpu.SemaphoreType.DMA((2,)),
                pltpu.SemaphoreType.DMA((2 * NCB,)),
                pltpu.SemaphoreType.DMA((NOUT, NCB)),
                pltpu.SemaphoreType.DMA((2, NBUF)),
            ],
            compiler_params=pltpu.CompilerParams(vmem_limit_bytes=64 * 1024 * 1024,
                                                 disable_bounds_checks=True),
        )(A_x.reshape(B, D), A_k, A_v, A_wq, A_wo.T, B_x.reshape(B, D), B_k, B_v, B_wq, B_wo.T)
        return out.reshape(B, Sq, 2 * D)
    return fn


@jax.jit
def pallas_concat_heads__sliding_block_cached__sliding_block_cached__decode_kernel(
    A_x, A_k_cache, A_v_cache, A_wq, A_wo, B_x, B_k_cache, B_v_cache, B_wq, B_wo):
    return make()(A_x, A_k_cache, A_v_cache, A_wq, A_wo, B_x, B_k_cache, B_v_cache, B_wq, B_wo)
```

```python
import jax
import jax.numpy as jnp
from jax import lax
import jax.experimental.pallas as pl
import jax.experimental.pallas.tpu as pltpu

_HQ, _DH = 32, 128
_F = _HQ * _DH

_NN = (((1,), (0,)), ((), ()))
_NT = (((1,), (1,)), ((), ()))

_ROWS = 128
_SHIFT = 64
_W_COLS = ((0, 1024), (1024, 2048), (3072, 1024))
_TAIL = _W_COLS[-1][1]
_Q_COLS = 1024
_SLOTS = 3
_UNIT = 4
_LAND = 3


def _div(a, n):
    return lax.div(a, jnp.int32(n))


def _rem(a, n):
    return lax.rem(a, jnp.int32(n))


def _dispatch(i, lo, hi, fn):
    pl.when(jnp.logical_and(i >= lo, i < hi))(lambda: fn(jnp.maximum(i - lo, 0)))


def _wait_filled(buf, sem):
    pltpu.make_async_copy(buf, buf, sem).wait()


def _kernel(ax, ak, av, awq, awo, bx, bk, bv, bwq, bwo, o_ref,
            x_buf, wq_buf, wo_buf, kv_buf, q_buf, att_buf, res_buf,
            kv_sem, wq_sem, wo_sem, aux_sem):
    batch, d_model = ax.shape
    hkv, sk = ak.shape[1], ak.shape[2]
    window = kv_buf.shape[3]
    caches = (ak, av, bk, bv)
    n_chunks = window // _ROWS

    n_q = 2 * _F // _Q_COLS
    n_att = 2 * batch * hkv
    n_w = d_model // 64
    kv_0, wo_0, n_steps = n_w, n_w + n_att, 2 * n_w + n_att
    last = n_w - 1

    def unit_of(i):
        unit = _div(i, _UNIT)
        return _rem(unit, _SLOTS), _div(unit, hkv // 2), 2 * _rem(unit, hkv // 2)

    x_copies = [pltpu.make_async_copy(x, x_buf.at[i], aux_sem) for i, x in enumerate((ax, bx))]

    def start_wq(s):
        @pl.loop(0, 2)
        def _(half):
            for c, n in _W_COLS:
                for stream in range(4):
                    rows = pl.ds(pl.multiple_of(stream * (d_model // 4) + s * 16 + half * 8, 8), 8)
                    for br, wq in enumerate((awq, bwq)):
                        pltpu.make_async_copy(
                            wq.at[rows, pl.ds(c, n)], wq_buf.at[br, rows, pl.ds(c, n)], wq_sem
                        ).start(priority=br)

    def start_kv(s):
        slot, b, h0 = unit_of(s)

        def fetch(g, row, n):
            for a, cache in enumerate(caches):
                pltpu.make_async_copy(
                    cache.at[b, h0 + g, pl.ds(sk - window + row, n), :],
                    kv_buf.at[slot, g, a, pl.ds(row, n), :],
                    kv_sem.at[slot],
                ).start(priority=a % 2)

        @pl.loop(0, n_chunks // _UNIT)
        def _(j):
            chunk = _rem(s, _UNIT) * (n_chunks // _UNIT) + j

            @pl.when(chunk < n_chunks - 1)
            def _():
                for g in range(2):
                    fetch(g, pl.multiple_of(chunk * _ROWS + _SHIFT, _SHIFT), _ROWS)

            @pl.when(chunk == n_chunks - 1)
            def _():
                for g in range(2):
                    fetch(g, 0, _SHIFT)
                    fetch(g, window - _ROWS + _SHIFT, _ROWS - _SHIFT)

    def start_wo(t):
        for c, n in _W_COLS:
            is_tail = c >= _F - _TAIL
            sem = wo_sem.at[jnp.where(t == last, n_w, t) if is_tail else t]
            for r in (0, 16, 32, 48, 8, 24, 40, 56):
                for br, wo in enumerate((awo, bwo)):
                    src_rows = pl.ds(pl.multiple_of(t * 64 + r, 8), 8)
                    dst_rows = pl.ds(pl.multiple_of(_rem(t + br, 2) * 64 + r, 8), 8)
                    pltpu.make_async_copy(
                        wo.at[src_rows, pl.ds(c, n)], wo_buf.at[t, dst_rows, pl.ds(c, n)], sem
                    ).start(priority=1 if is_tail else br)

    def q_task(i):
        @pl.when(i == 0)
        def _():
            for copy in x_copies:
                copy.wait()
            _wait_filled(wq_buf, wq_sem)

        br, c = _div(i, _F // _Q_COLS), _rem(i, _F // _Q_COLS)
        w = wq_buf[br, :, pl.ds(pl.multiple_of(c * _Q_COLS, _Q_COLS), _Q_COLS)]
        q = lax.dot_general(x_buf[br], w, _NN, preferred_element_type=jnp.float32)
        for j in range(_Q_COLS // _DH):
            q_buf[br, c * (_Q_COLS // _DH) + j] = q[:, j * _DH:(j + 1) * _DH]

    def attention_task(i):
        slot, b, h0 = unit_of(i)
        part = _rem(i, _UNIT)
        g, br = _div(part, 2), _rem(part, 2)
        head = 2 * (h0 + g)

        @pl.when(part == 0)
        def _():
            _wait_filled(kv_buf.at[slot], kv_sem.at[slot])

        q0 = jnp.broadcast_to(q_buf[br, head, pl.ds(b, 1), :], (8, _DH))
        q1 = jnp.broadcast_to(q_buf[br, head + 1, pl.ds(b, 1), :], (8, _DH))
        q = jnp.where(lax.broadcasted_iota(jnp.int32, (8, _DH), 0) < 4, q0, q1)
        k = kv_buf[slot, g, 2 * br]
        v = kv_buf[slot, g, 2 * br + 1]
        s = lax.dot_general(q.astype(k.dtype), k, _NT, preferred_element_type=jnp.float32)
        s = s * (_DH ** -0.5)
        p = jnp.exp(s - jnp.max(s, axis=-1, keepdims=True))
        o = lax.dot_general(p.astype(v.dtype), v, _NN, preferred_element_type=jnp.float32)
        o = o / jnp.sum(p, axis=-1, keepdims=True)
        att_buf[head, pl.ds(br * batch + b, 1), :] = o[0:1]
        att_buf[head + 1, pl.ds(br * batch + b, 1), :] = o[4:5]

    def project(t, lo, hi):
        att = jnp.concatenate([att_buf[h] for h in range(lo // _DH, hi // _DH)], axis=1)
        w = wo_buf[t, :, pl.ds(lo, hi - lo)]
        return lax.dot_general(att.astype(w.dtype), w, _NT, preferred_element_type=jnp.float32)

    def projection_task(t):
        _wait_filled(wo_buf.at[t], wo_sem.at[t])
        res_buf[t] = project(t, 0, _F)

    n_tasks = n_q + n_att + last

    def step(s, done):
        _dispatch(s, 0, kv_0, start_wq)
        _dispatch(s, kv_0, wo_0, start_kv)
        _dispatch(s, wo_0, n_steps, start_wo)

        @pl.when(s == 0)
        def _():
            for copy in x_copies:
                copy.start()

        q_cap = 2 * (s - (kv_0 - 2 + _LAND))
        att_cap = n_q + s - kv_0 - (_UNIT - 2 + _LAND) + jnp.maximum(0, s - (wo_0 - 2 + _LAND))
        proj_cap = n_q + n_att + jnp.maximum(0, s - wo_0 - 1)
        target = jnp.maximum(jnp.minimum(jnp.minimum(q_cap, att_cap), proj_cap), 0)
        target = jnp.where(s == n_steps - 1, n_tasks, target)

        @pl.loop(done, target)
        def _(i):
            _dispatch(i, 0, n_q, q_task)
            _dispatch(i, n_q, n_q + n_att, attention_task)
            _dispatch(i, n_q + n_att, n_tasks, projection_task)

        return target

    lax.fori_loop(0, n_steps, step, jnp.int32(0))

    def write_tile(n, last_res=None):
        def columns(j):
            br, t = divmod(j, n_w)
            res = last_res if t == last else res_buf[t]
            return res[br * batch:(br + 1) * batch]

        lane = lax.broadcasted_iota(jnp.int32, (batch, 128), 1)
        tile = jnp.where(lane < 64, columns(2 * n), columns(2 * n + 1))
        o_ref[:, pl.ds(n * 128, 128)] = tile.astype(o_ref.dtype)

    late_tiles = (last // 2, (n_w + last) // 2)
    for n in range(n_w):
        if n not in late_tiles:
            write_tile(n)
    _wait_filled(wo_buf.at[last, :, pl.ds(0, _F - _TAIL)], wo_sem.at[last])
    res_buf[last] = project(last, 0, _F - _TAIL)
    _wait_filled(wo_buf.at[last, :, pl.ds(_F - _TAIL, _TAIL)], wo_sem.at[n_w])
    last_res = res_buf[last] + project(last, _F - _TAIL, _F)
    for n in late_tiles:
        write_tile(n, last_res)


@jax.jit
def pallas_concat_heads__sliding_block_cached__sliding_block_cached__decode_kernel(
    A_x: jax.Array,
    A_k_cache: jax.Array,
    A_v_cache: jax.Array,
    A_wq: jax.Array,
    A_wo: jax.Array,
    B_x: jax.Array,
    B_k_cache: jax.Array,
    B_v_cache: jax.Array,
    B_wq: jax.Array,
    B_wo: jax.Array,
):
    batch, sq, d_model = A_x.shape
    hkv, sk = A_k_cache.shape[1], A_k_cache.shape[2]
    window = min(4096, max(256, sk // 4))
    assert (batch, sq, d_model, 2 * hkv) == (4, 1, 576, _HQ)
    assert window % (_ROWS * _UNIT) == 0
    n_w = d_model // 64

    out = pl.pallas_call(
        _kernel,
        out_shape=jax.ShapeDtypeStruct((batch, 2 * d_model), A_x.dtype),
        in_specs=[pl.BlockSpec(memory_space=pltpu.HBM)] * 10,
        out_specs=pl.BlockSpec(memory_space=pltpu.VMEM),
        scratch_shapes=[
            pltpu.VMEM((2, batch, d_model), A_x.dtype),
            pltpu.VMEM((2, d_model, _F), A_wq.dtype),
            pltpu.VMEM((n_w, 128, _F), A_wo.dtype),
            pltpu.VMEM((_SLOTS, 2, 4, window, _DH), A_k_cache.dtype),
            pltpu.VMEM((2, _HQ, batch, _DH), jnp.float32),
            pltpu.VMEM((_HQ, 2 * batch, _DH), jnp.float32),
            pltpu.VMEM((n_w, 2 * batch, 128), jnp.float32),
            pltpu.SemaphoreType.DMA((_SLOTS,)),
            pltpu.SemaphoreType.DMA(()),
            pltpu.SemaphoreType.DMA((n_w + 1,)),
            pltpu.SemaphoreType.DMA(()),
        ],
        compiler_params=pltpu.CompilerParams(
            vmem_limit_bytes=64 * 1024 * 1024,
            disable_bounds_checks=True,
            disable_semaphore_checks=True,
        ),
    )(
        A_x.reshape(batch, d_model), A_k_cache, A_v_cache, A_wq, A_wo.T,
        B_x.reshape(batch, d_model), B_k_cache, B_v_cache, B_wq, B_wo.T,
    )
    return out.reshape(batch, sq, 2 * d_model)
```

```python
import jax
import jax.numpy as jnp
from jax import lax
import jax.experimental.pallas as pl
import jax.experimental.pallas.tpu as pltpu
import numpy as np

_HQ, _DH = 32, 128
_F = _HQ * _DH

_NN = (((1,), (0,)), ((), ()))
_NT = (((1,), (1,)), ((), ()))

_ROWS = 128
_SHIFT = 64
_W_COLS = ((0, 1024), (1024, 2048), (3072, 1024))
_HEAD, _TAIL = _W_COLS[-1]
_Q_COLS = 1024
_SLOTS = 3
_UNIT = 4
_LAND = 3


def _div(a, n):
    return lax.div(a, np.int32(n))


def _rem(a, n):
    return lax.rem(a, np.int32(n))


def _dispatch(i, lo, hi, fn):
    pl.when(jnp.logical_and(i >= lo, i < hi))(lambda: fn(jnp.maximum(i - lo, 0)))


def _wait_filled(buf, sem):
    pltpu.make_async_copy(buf, buf, sem).wait()


def _kernel(ax, ak, av, awq, awo, bx, bk, bv, bwq, bwo, o_ref,
            x_buf, wq_buf, wo_head, wo_tail, kv_buf, q_buf, att_buf, res_buf,
            kv_sem, wq_sem, wo_sem, aux_sem):
    batch, d_model = ax.shape
    hkv, sk = ak.shape[1], ak.shape[2]
    window = kv_buf.shape[3]
    caches = (ak, av, bk, bv)
    n_chunks = window // _ROWS

    n_q = 2 * _F // _Q_COLS
    n_att = 2 * batch * hkv
    n_w = d_model // 64
    kv_0, wo_0, n_steps = n_w, n_w + n_att, 2 * n_w + n_att
    last = n_w - 1

    def unit_of(i):
        unit = _div(i, _UNIT)
        return _rem(unit, _SLOTS), _div(unit, hkv // 2), 2 * _rem(unit, hkv // 2)

    x_copies = [pltpu.make_async_copy(x, x_buf.at[i], aux_sem) for i, x in enumerate((ax, bx))]

    def start_wq(s):
        @pl.loop(0, 2)
        def _(half):
            for c, n in _W_COLS:
                for stream in range(4):
                    rows = pl.ds(pl.multiple_of(stream * (d_model // 4) + s * 16 + half * 8, 8), 8)
                    for br, wq in enumerate((awq, bwq)):
                        pltpu.make_async_copy(
                            wq.at[rows, pl.ds(c, n)], wq_buf.at[br, rows, pl.ds(c, n)], wq_sem
                        ).start(priority=br)

    def start_kv(s):
        slot, b, h0 = unit_of(s)

        def fetch(g, row, n):
            for a, cache in enumerate(caches):
                pltpu.make_async_copy(
                    cache.at[b, h0 + g, pl.ds(sk - window + row, n), :],
                    kv_buf.at[slot, g, a, pl.ds(row, n), :],
                    kv_sem.at[slot],
                ).start(priority=a % 2)

        @pl.loop(0, n_chunks // _UNIT)
        def _(j):
            chunk = _rem(s, _UNIT) * (n_chunks // _UNIT) + j

            @pl.when(chunk < n_chunks - 1)
            def _():
                for g in range(2):
                    fetch(g, pl.multiple_of(chunk * _ROWS + _SHIFT, _SHIFT), _ROWS)

            @pl.when(chunk == n_chunks - 1)
            def _():
                for g in range(2):
                    fetch(g, 0, _SHIFT)
                    fetch(g, window - _ROWS + _SHIFT, _ROWS - _SHIFT)

    def start_wo(t):
        for c, n in _W_COLS:
            is_tail = c >= _HEAD
            sem = wo_sem.at[jnp.where(t == last, n_w, t) if is_tail else t]
            for r in (0, 16, 32, 48, 8, 24, 40, 56):
                for br, wo in enumerate((awo, bwo)):
                    src_rows = pl.ds(pl.multiple_of(t * 64 + r, 8), 8)
                    dst_rows = pl.ds(pl.multiple_of(_rem(t + br, 2) * 64 + r, 8), 8)
                    dst = wo_tail.at[t, dst_rows] if is_tail else wo_head.at[t, dst_rows, pl.ds(c, n)]
                    pltpu.make_async_copy(wo.at[src_rows, pl.ds(c, n)], dst, sem).start(
                        priority=1 if is_tail else br)

    def q_task(i):
        @pl.when(i == 0)
        def _():
            for copy in x_copies:
                copy.wait()
            _wait_filled(wq_buf, wq_sem)

        br, c = _div(i, _F // _Q_COLS), _rem(i, _F // _Q_COLS)
        w = wq_buf[br, :, pl.ds(pl.multiple_of(c * _Q_COLS, _Q_COLS), _Q_COLS)]
        q = lax.dot_general(x_buf[br], w, _NN, preferred_element_type=jnp.float32)
        for j in range(_Q_COLS // _DH):
            q_buf[br, c * (_Q_COLS // _DH) + j] = q[:, j * _DH:(j + 1) * _DH]

    def attention_task(i):
        slot, b, h0 = unit_of(i)
        part = _rem(i, _UNIT)
        g, br = _div(part, 2), _rem(part, 2)
        head = 2 * (h0 + g)

        @pl.when(part == 0)
        def _():
            _wait_filled(kv_buf.at[slot], kv_sem.at[slot])

        q0 = jnp.broadcast_to(q_buf[br, head, pl.ds(b, 1), :], (8, _DH))
        q1 = jnp.broadcast_to(q_buf[br, head + 1, pl.ds(b, 1), :], (8, _DH))
        q = jnp.where(lax.broadcasted_iota(jnp.int32, (8, _DH), 0) < 4, q0, q1)
        k = kv_buf[slot, g, 2 * br]
        v = kv_buf[slot, g, 2 * br + 1]
        s = lax.dot_general(q.astype(k.dtype), k, _NT, preferred_element_type=jnp.float32)
        s = s * (_DH ** -0.5)
        p = jnp.exp(s - jnp.max(s, axis=-1, keepdims=True))
        o = lax.dot_general(p.astype(v.dtype), v, _NN, preferred_element_type=jnp.float32)
        o = o / jnp.sum(p, axis=-1, keepdims=True)
        att_buf[head, pl.ds(br * batch + b, 1), :] = o[0:1]
        att_buf[head + 1, pl.ds(br * batch + b, 1), :] = o[4:5]

    def project(w, lo):
        heads = range(lo // _DH, (lo + w.shape[1]) // _DH)
        att = jnp.concatenate([att_buf[h] for h in heads], axis=1)
        return lax.dot_general(att.astype(w.dtype), w, _NT, preferred_element_type=jnp.float32)

    def projection_task(t):
        _wait_filled(wo_head.at[t], wo_sem.at[t])
        _wait_filled(wo_tail.at[t], wo_sem.at[t])
        res_buf[t] = project(wo_head[t], 0) + project(wo_tail[t], _HEAD)

    n_tasks = n_q + n_att + last

    def step(s, done):
        _dispatch(s, 0, kv_0, start_wq)
        _dispatch(s, kv_0, wo_0, start_kv)
        _dispatch(s, wo_0, n_steps, start_wo)

        @pl.when(s == 0)
        def _():
            for copy in x_copies:
                copy.start()

        q_cap = 2 * (s - (kv_0 - 2 + _LAND))
        att_cap = n_q + s - kv_0 - (_UNIT - 2 + _LAND) + jnp.maximum(0, s - (wo_0 - 2 + _LAND))
        proj_cap = n_q + n_att + jnp.maximum(0, s - wo_0 - 1)
        target = jnp.maximum(jnp.minimum(jnp.minimum(q_cap, att_cap), proj_cap), 0)
        target = jnp.where(s == n_steps - 1, n_tasks, target)

        @pl.loop(done, target)
        def _(i):
            _dispatch(i, 0, n_q, q_task)
            _dispatch(i, n_q, n_q + n_att, attention_task)
            _dispatch(i, n_q + n_att, n_tasks, projection_task)

        return target

    lax.fori_loop(0, n_steps, step, np.int32(0))

    def write_tile(n, last_res=None):
        def columns(j):
            br, t = divmod(j, n_w)
            res = last_res if t == last else res_buf[t]
            return res[br * batch:(br + 1) * batch]

        lane = lax.broadcasted_iota(jnp.int32, (batch, 128), 1)
        tile = jnp.where(lane < 64, columns(2 * n), columns(2 * n + 1))
        o_ref[:, pl.ds(n * 128, 128)] = tile.astype(o_ref.dtype)

    late_tiles = (last // 2, (n_w + last) // 2)
    for n in range(n_w):
        if n not in late_tiles:
            write_tile(n)
    _wait_filled(wo_head.at[last], wo_sem.at[last])
    res_buf[last] = project(wo_head[last], 0)
    _wait_filled(wo_tail.at[last], wo_sem.at[n_w])
    last_res = res_buf[last] + project(wo_tail[last], _HEAD)
    for n in late_tiles:
        write_tile(n, last_res)


@jax.jit
def pallas_concat_heads__sliding_block_cached__sliding_block_cached__decode_kernel(
    A_x: jax.Array,
    A_k_cache: jax.Array,
    A_v_cache: jax.Array,
    A_wq: jax.Array,
    A_wo: jax.Array,
    B_x: jax.Array,
    B_k_cache: jax.Array,
    B_v_cache: jax.Array,
    B_wq: jax.Array,
    B_wo: jax.Array,
):
    batch, sq, d_model = A_x.shape
    hkv, sk = A_k_cache.shape[1], A_k_cache.shape[2]
    window = min(4096, max(256, sk // 4))
    assert (batch, sq, d_model, 2 * hkv) == (4, 1, 576, _HQ)
    assert window % (_ROWS * _UNIT) == 0
    n_w = d_model // 64

    out = pl.pallas_call(
        _kernel,
        out_shape=jax.ShapeDtypeStruct((batch, 2 * d_model), A_x.dtype),
        in_specs=[pl.BlockSpec(memory_space=pltpu.HBM)] * 10,
        out_specs=pl.BlockSpec(memory_space=pltpu.VMEM),
        scratch_shapes=[
            pltpu.VMEM((2, batch, d_model), A_x.dtype),
            pltpu.VMEM((2, d_model, _F), A_wq.dtype),
            pltpu.VMEM((n_w, 128, _HEAD), A_wo.dtype),
            pltpu.VMEM((n_w, 128, _TAIL), A_wo.dtype),
            pltpu.VMEM((_SLOTS, 2, 4, window, _DH), A_k_cache.dtype),
            pltpu.VMEM((2, _HQ, batch, _DH), jnp.float32),
            pltpu.VMEM((_HQ, 2 * batch, _DH), jnp.float32),
            pltpu.VMEM((n_w, 2 * batch, 128), jnp.float32),
            pltpu.SemaphoreType.DMA((_SLOTS,)),
            pltpu.SemaphoreType.DMA(()),
            pltpu.SemaphoreType.DMA((n_w + 1,)),
            pltpu.SemaphoreType.DMA(()),
        ],
        compiler_params=pltpu.CompilerParams(
            vmem_limit_bytes=64 * 1024 * 1024,
            disable_bounds_checks=True,
            disable_semaphore_checks=True,
        ),
    )(
        A_x.reshape(batch, d_model), A_k_cache, A_v_cache, A_wq, A_wo.T,
        B_x.reshape(batch, d_model), B_k_cache, B_v_cache, B_wq, B_wo.T,
    )
    return out.reshape(batch, sq, 2 * d_model)
```
